```python
import os as _os
_os.environ.setdefault("JAX_PLATFORMS", "cpu")
import jax
import jax.numpy as jnp

def _softmax(x, axis=-1):
    return jax.nn.softmax(x, axis=axis)
def _gelu(x):
    return jax.nn.gelu(x, approximate=True)
def _silu(x):
    return jax.nn.silu(x)
def _sigmoid(x):
    return jax.nn.sigmoid(x)
def _layernorm(x, axis=-1, eps=1e-5):
    m = jnp.mean(x, axis=axis, keepdims=True)
    v = jnp.var(x, axis=axis, keepdims=True)
    return (x - m) / jnp.sqrt(v + eps)
def _scatter_add(tgt, idx, src, axis=0):
    return tgt.at[idx].add(src)
def _segment_sum(src, seg, n):
    return jax.ops.segment_sum(src, seg, n)
class _Rng:
    def __init__(self, key):
        self._k = key
    def _next(self):
        self._k, sub = jax.random.split(self._k)
        return sub
    def normal(self, shape):
        return jax.random.normal(self._next(), shape, dtype=jnp.bfloat16)
    def randint(self, lo, hi, shape):
        return jax.random.randint(self._next(), shape, lo, hi, dtype=jnp.int32)
    def uniform(self, shape, lo=0.0, hi=1.0):
        return jax.random.uniform(self._next(), shape, jnp.bfloat16, lo, hi)
    def permutation(self, n):
        return jax.random.permutation(self._next(), n)


kernel_name = 'interleave_layers__sliding_block__dense_activation_gelu__prompt'

def setup_inputs():
    _rng = _Rng(jax.random.key(int.from_bytes(__import__("os").urandom(4), "little")))
    _w = (lambda a: (lambda t: t.astype(jnp.bfloat16) if jnp.issubdtype(t.dtype, jnp.floating) else t)(jnp.asarray(a)))
    def _A_setup():
        B, S, D = 1, 2048, 640
        return {
            "x": _w((lambda *s: _rng.normal(s) * 0.05)(B, S, D)),
            "wqkv": _w((lambda *s: _rng.normal(s) * 0.05)(D, 3 * D)),
            "wo": _w((lambda *s: _rng.normal(s) * 0.05)(D, D)),
        }
    _A_in = _A_setup()

    def _B_setup():
        B, S, D, F = 1, 2048, 640, 1728
        return {
            "x": _w((lambda *s: _rng.normal(s) * 0.05)(B, S, D)),
            "w1": _w((lambda *s: _rng.normal(s) * 0.8)(D, F) * (D ** -0.5)),
            "b1": _w((lambda *s: _rng.normal(s) * 0.8)(F) * 0.01),
            "w2": _w((lambda *s: _rng.normal(s) * 0.8)(F, D) * (F ** -0.5)),
            "b2": _w((lambda *s: _rng.normal(s) * 0.8)(D) * 0.01),
        }
    _B_in = _B_setup()

    return {
        "A_x": _A_in["x"],
        "A_wqkv": _A_in["wqkv"],
        "A_wo": _A_in["wo"],
        "B_x": _B_in["x"],
        "B_w1": _B_in["w1"],
        "B_b1": _B_in["b1"],
        "B_w2": _B_in["w2"],
        "B_b2": _B_in["b2"],
    }

def reference(A_x, A_wqkv, A_wo, B_x, B_w1, B_b1, B_w2, B_b2):
    def _A_ref(x, wqkv, wo):
        B, S, D = x.shape
        H = 32; Dh = D // H; W = 256
        qkv = (lambda x, *d: x.transpose(*d))((x @ wqkv).reshape(B, S, 3, H, Dh), 2, 0, 3, 1, 4)
        q, k, v = qkv[0], qkv[1], qkv[2]
        scores = jnp.einsum("bhqd,bhkd->bhqk", q, k) * (Dh ** -0.5)
        idx = jnp.arange(S)
        mask = (idx[:, None] - idx[None, :] >= 0) & (idx[:, None] - idx[None, :] < W)
        scores = jnp.where(mask[None, None], scores, -1e9)
        p = _softmax(scores, axis=-1)
        o = jnp.einsum("bhqk,bhkd->bhqd", p, v)
        return (lambda x, *d: x.transpose(*d))(o, 0, 2, 1, 3).reshape(B, S, D) @ wo

    def _B_ref(x, w1, b1, w2, b2):
        h = jnp.einsum("bsd,df->bsf", x, w1) + b1
        h = _gelu(h)
        return jnp.einsum("bsf,fd->bsd", h, w2) + b2

    x = A_x
    x = x + _A_ref(_layernorm(x, axis=-1), A_wqkv, A_wo)
    x = x + _B_ref(_layernorm(x, axis=-1), B_w1, B_b1, B_w2, B_b2)
    x = x + _A_ref(_layernorm(x, axis=-1), A_wqkv, A_wo)
    x = x + _B_ref(_layernorm(x, axis=-1), B_w1, B_b1, B_w2, B_b2)
    return x
```

```python
import functools
import numpy as np
import jax
import jax.numpy as jnp
from jax import lax
import jax.experimental.pallas as pl
import jax.experimental.pallas.tpu as pltpu

_H = 32
_W = 256
_QB = 128
_R = 512
_NEG = -1e30
_GB = 4


def _layernorm(x):
    m = jnp.mean(x, axis=-1, keepdims=True)
    xc = x - m
    v = jnp.mean(xc * xc, axis=-1, keepdims=True)
    return xc * lax.rsqrt(v + 1e-5)


def _gelu(x):
    c = float(np.sqrt(2.0 / np.pi))
    return 0.5 * x * (1.0 + jnp.tanh(c * (x + 0.044715 * (x * x * x))))


def _dot(a, b):
    return jnp.dot(a, b, preferred_element_type=jnp.float32)


def _dot_nt(a, b):
    return lax.dot_general(a, b, (((1,), (1,)), ((), ())),
                           preferred_element_type=jnp.float32)


def _kernel(x_ref, wqkv_hbm, wo_hbm, w1t_hbm, b1_ref, w2_hbm, b2_ref, o_ref,
            k_scr, vt_scr, wqkv_ref, wo_ref, w1t_ref, w2_ref, sems, *, D, Dh):
    step = pl.program_id(0)
    G = 4 * Dh
    NG = D // G
    SB = _QB // 4
    NK = _W + SB

    copies = [pltpu.make_async_copy(src, dst, sems.at[i]) for i, (src, dst) in enumerate(
        [(wqkv_hbm, wqkv_ref), (wo_hbm, wo_ref), (w1t_hbm, w1t_ref), (w2_hbm, w2_ref)])]

    @pl.when(step == 0)
    def _():
        for c in copies:
            c.start()
        lane = lax.broadcasted_iota(jnp.int32, (2, _W, NG * 128), 2)
        k_scr[:, 0:_W, :] = jnp.where(lane % 128 == G, 1.0, 0.0).astype(jnp.bfloat16)
        vt_scr[:, :, 0:_W] = jnp.zeros((2, D, _W), jnp.bfloat16)
        copies[0].wait()

    qscale = float(Dh ** -0.5 * np.log2(np.e))
    row0 = pl.multiple_of(step * _R, _R)

    sub = lax.broadcasted_iota(jnp.int32, (8, _QB), 0)
    upper = sub < 4
    er = lax.broadcasted_iota(jnp.int32, (_QB, _QB), 0)
    eq = lax.broadcasted_iota(jnp.int32, (_QB, _QB), 1)
    causal = er <= eq
    causal_f = jnp.where(causal, 1.0, 0.0)
    padrow = lax.broadcasted_iota(jnp.int32, (128 - G, _QB), 0)
    qpad = jnp.where(padrow == 0, _NEG, 0.0)
    zslab = jnp.zeros((8, _QB), jnp.float32)

    def attention(q, layer, qb):
        kstart = pl.multiple_of(row0 + qb * _QB, _QB)
        qt = q.T
        vt = vt_scr[layer, :, pl.ds(kstart, 3 * _QB)]
        oslabs = [None] * (D // 8)
        for g0 in range(0, NG, _GB):
            ss = []
            for g in range(g0, g0 + _GB):
                cols = []
                for h in range(4 * g, 4 * g + 4):
                    lo, hi = h * Dh, (h + 1) * Dh
                    sl = []
                    for i in range(g * G // 8, (g + 1) * G // 8):
                        t = qt[8 * i:8 * i + 8]
                        if 8 * i + 8 <= lo or 8 * i >= hi:
                            t = zslab
                        elif 8 * i < lo:
                            t = jnp.where(upper, 0.0, t)
                        elif 8 * i + 8 > hi:
                            t = jnp.where(upper, t, 0.0)
                        sl.append(t)
                    cols.append(jnp.concatenate(sl + [qpad], axis=0))
                rhs = jnp.concatenate(cols, axis=1).astype(jnp.bfloat16)
                kt = k_scr[layer, pl.ds(kstart, 3 * _QB), 128 * g:128 * (g + 1)]
                kt = jnp.concatenate([kt[0:_QB], kt[2 * _QB:], kt[_QB:2 * _QB]], axis=0)
                ss.append(_dot(kt, rhs))
            ps, ls = [], []
            for hh in range(4 * _GB):
                s = ss[hh // 4][:, (hh % 4) * _QB:(hh % 4 + 1) * _QB]
                s_c = jnp.where(causal, s[_QB:2 * _QB], s[0:_QB])
                s_m = s[2 * _QB:]
                m = jnp.max(jnp.maximum(s_c, s_m), axis=0, keepdims=True)
                p_c = jnp.exp2(s_c - m)
                p_m = jnp.exp2(s_m - m)
                ls.append(1.0 / jnp.sum(p_c + p_m, axis=0, keepdims=True))
                p_d = p_c * causal_f
                ps.append(jnp.concatenate([p_c - p_d, p_m, p_d], axis=0).astype(jnp.bfloat16))
            for hh in range(4 * _GB):
                h = 4 * g0 + hh
                lo, hi = h * Dh, (h + 1) * Dh
                w0 = (lo // 16) * 16
                o = _dot(vt[w0:w0 + 32], ps[hh]) * ls[hh]
                for i in range(lo // 8, (hi + 7) // 8):
                    t = o[8 * i - w0:8 * i - w0 + 8]
                    if 8 * i < lo:
                        t = jnp.where(upper, oslabs[i], t)
                    oslabs[i] = t
        return jnp.concatenate(oslabs, axis=0).T

    def layer_body(layer, x):
        xn = _layernorm(x).astype(jnp.bfloat16)
        qkv = _dot(xn, wqkv_ref[...])
        q = qkv[:, 0:D] * qscale
        k = qkv[:, D:2 * D]
        v = qkv[:, 2 * D:]
        zk = jnp.zeros((_R, 128 - G), jnp.float32)
        kparts = []
        for g in range(NG):
            kparts += [k[:, g * G:(g + 1) * G], zk]
        k = jnp.concatenate(kparts, axis=1)
        wstart = pl.multiple_of(row0 + _W, _QB)
        k_scr[layer, pl.ds(wstart, _R), :] = k.astype(jnp.bfloat16)
        vt_scr[layer, :, pl.ds(wstart, _R)] = v.T.astype(jnp.bfloat16)
        o = jnp.concatenate(
            [attention(q[qb * _QB:(qb + 1) * _QB], layer, qb)
             for qb in range(_R // _QB)], axis=0)

        @pl.when((step == 0) & (layer == 0))
        def _():
            for c in copies[1:]:
                c.wait()
        x = x + _dot(o.astype(jnp.bfloat16), wo_ref[...])
        xn = _layernorm(x).astype(jnp.bfloat16)
        h = _gelu(_dot_nt(xn, w1t_ref[...]) + b1_ref[...].astype(jnp.float32).reshape(1, -1))
        return x + _dot(h.astype(jnp.bfloat16), w2_ref[...]) + b2_ref[...].astype(jnp.float32).reshape(1, -1)

    x = x_ref[...].astype(jnp.float32)
    x = lax.fori_loop(0, 2, layer_body, x)
    o_ref[...] = x.astype(o_ref.dtype)


@jax.jit
def pallas_interleave_layers__sliding_block__dense_activation_gelu__prompt_kernel(
    A_x, A_wqkv, A_wo, B_x, B_w1, B_b1, B_w2, B_b2,
):
    del B_x
    B, S, D = A_x.shape
    F = B_w1.shape[1]
    Dh = D // _H
    x2 = A_x.reshape(B * S, D)
    const = lambda i: (0, 0)
    wspec = lambda shape: pl.BlockSpec(shape, const, pipeline_mode=pl.Buffered(1))
    hbm = pl.BlockSpec(memory_space=pl.ANY)
    out = pl.pallas_call(
        functools.partial(_kernel, D=D, Dh=Dh),
        grid=(S // _R,),
        in_specs=[
            pl.BlockSpec((_R, D), lambda i: (i, 0)),
            hbm, hbm, hbm, pl.BlockSpec((F,), lambda i: (0,)), hbm, pl.BlockSpec((D,), lambda i: (0,)),
        ],
        out_specs=pl.BlockSpec((_R, D), lambda i: (i, 0)),
        out_shape=jax.ShapeDtypeStruct((B * S, D), A_x.dtype),
        scratch_shapes=[pltpu.VMEM((2, S + _W, 2 * 4 * 128), jnp.bfloat16),
                        pltpu.VMEM((2, D, S + _W), jnp.bfloat16),
                        pltpu.VMEM((D, 3 * D), jnp.bfloat16), pltpu.VMEM((D, D), jnp.bfloat16),
                        pltpu.VMEM((F, D), jnp.bfloat16), pltpu.VMEM((F, D), jnp.bfloat16),
                        pltpu.SemaphoreType.DMA((4,))],
        compiler_params=pltpu.CompilerParams(
            dimension_semantics=("arbitrary",), flags={"XLA_TPU_FORCE_LP_LLO_SCHEDULER": True},
            vmem_limit_bytes=100 * 1024 * 1024),
    )(x2, A_wqkv, A_wo, B_w1.T, B_b1, B_w2, B_b2)
    return out.reshape(B, S, D)
```
